```python
import os as _os
_os.environ.setdefault('JAX_PLATFORMS', 'cpu')
import jax
import jax.numpy as jnp

def _softmax(x, axis=-1):
    return jax.nn.softmax(x, axis=axis)

def _gelu(x):
    return jax.nn.gelu(x, approximate=True)

def _silu(x):
    return jax.nn.silu(x)

def _sigmoid(x):
    return jax.nn.sigmoid(x)

def _layernorm(x, axis=-1, eps=1e-05):
    m = jnp.mean(x, axis=axis, keepdims=True)
    v = jnp.var(x, axis=axis, keepdims=True)
    return (x - m) / jnp.sqrt(v + eps)

def _scatter_add(tgt, idx, src, axis=0):
    return tgt.at[idx].add(src)

def _segment_sum(src, seg, n):
    return jax.ops.segment_sum(src, seg, n)

class _Rng:

    def __init__(self, key):
        self._k = key

    def _next(self):
        self._k, sub = jax.random.split(self._k)
        return sub

    def normal(self, shape):
        return jax.random.normal(self._next(), shape, dtype=jnp.bfloat16)

    def randint(self, lo, hi, shape):
        return jax.random.randint(self._next(), shape, lo, hi, dtype=jnp.int32)

    def uniform(self, shape, lo=0.0, hi=1.0):
        return jax.random.uniform(self._next(), shape, jnp.bfloat16, lo, hi)

    def permutation(self, n):
        return jax.random.permutation(self._next(), n)
kernel_name = 'gated_mix__memory_aug_recurrent_mem_tr__glu_gated_geglu__prompt'

def setup_inputs():
    _rng = _Rng(jax.random.key(int.from_bytes(__import__("os").urandom(4), "little")))
    _w = lambda a: (lambda t: t.astype(jnp.bfloat16) if jnp.issubdtype(t.dtype, jnp.floating) else t)(jnp.asarray(a))

    def _A_setup():
        B, S, Dm = (1, 2048, 640)
        H, Dh = (32, 128)
        M, seg = (8, 32)
        seg = min(seg, S)
        S = S // seg * seg
        return {'x': _w((lambda *s: _rng.normal(s) * 0.05)(B, S, Dm)), 'mem0': _w((lambda *s: _rng.normal(s) * 0.4)(B, M, Dm)), 'Wq': _w((lambda *s: _rng.normal(s) * 3.2)(Dm, H, Dh) * Dm ** (-0.5)), 'Wk': _w((lambda *s: _rng.normal(s) * 3.2)(Dm, H, Dh) * Dm ** (-0.5)), 'Wv': _w((lambda *s: _rng.normal(s) * 0.4)(Dm, H, Dh) * Dm ** (-0.5)), 'Wo': _w((lambda *s: _rng.normal(s) * 0.4)(H, Dh, Dm) * (H * Dh) ** (-0.5)), 'seg_len': seg}
    _A_in = _A_setup()

    def _B_setup():
        B, S, Dm, Df = (1, 2048, 640, 1728)
        return {'x': _w((lambda *s: _rng.normal(s) * 0.05)(B, S, Dm)), 'w_gate': _w((lambda *s: _rng.normal(s) * 1.6)(Dm, Df) * Dm ** (-0.5)), 'w_up': _w((lambda *s: _rng.normal(s) * 1.6)(Dm, Df) * Dm ** (-0.5)), 'w_down': _w((lambda *s: _rng.normal(s) * 1.6)(Df, Dm) * Df ** (-0.5))}
    _B_in = _B_setup()
    return {'A_x': _A_in['x'], 'A_mem0': _A_in['mem0'], 'A_Wq': _A_in['Wq'], 'A_Wk': _A_in['Wk'], 'A_Wv': _A_in['Wv'], 'A_Wo': _A_in['Wo'], 'A_seg_len': _A_in['seg_len'], 'B_x': _B_in['x'], 'B_w_gate': _B_in['w_gate'], 'B_w_up': _B_in['w_up'], 'B_w_down': _B_in['w_down'], 'gate_w': _w((lambda *s: _rng.normal(s) * 0.05)(640) * 16.0)}

def reference(A_x, A_mem0, A_Wq, A_Wk, A_Wv, A_Wo, A_seg_len, B_x, B_w_gate, B_w_up, B_w_down, gate_w):

    def _A_ref(x, mem0, Wq, Wk, Wv, Wo, seg_len):
        B, S, Dm = x.shape
        H, Dh = (Wq.shape[1], Wq.shape[2])
        M = mem0.shape[1]
        scale = Dh ** (-0.5)
        n_seg = S // seg_len
        L = M + seg_len
        idx = jnp.arange(L)
        mask = (idx[:, None] < M) | (idx[:, None] >= idx[None, :])
        mem = mem0
        outs = []
        for s in range(n_seg):
            xs = x[:, s * seg_len:(s + 1) * seg_len, :].copy()
            h = jnp.concatenate([mem, xs], axis=1)
            q = jnp.einsum('btd,dhe->bhte', h, Wq)
            k = jnp.einsum('btd,dhe->bhte', h, Wk)
            v = jnp.einsum('btd,dhe->bhte', h, Wv)
            scores = jnp.einsum('bhqe,bhke->bhqk', q, k) * scale
            scores = jnp.where(mask[None, None], scores, -1000000000.0)
            p = _softmax(scores, axis=-1)
            o = jnp.einsum('bhqk,bhke->bhqe', p, v)
            o = jnp.einsum('bhte,hed->btd', o, Wo)
            mem = o[:, :M, :].copy()
            outs.append(o[:, M:, :])
        return jnp.concatenate(outs, axis=1)

    def _B_ref(x, w_gate, w_up, w_down):
        g = jnp.einsum('bsd,df->bsf', x, w_gate)
        u = jnp.einsum('bsd,df->bsf', x, w_up)
        h = _gelu(g) * u
        return jnp.einsum('bsf,fd->bsd', h, w_down)
    x = A_x
    g = _sigmoid((x * gate_w).sum(-1, keepdims=True))
    a = _A_ref(x, A_mem0, A_Wq, A_Wk, A_Wv, A_Wo, A_seg_len)
    b = _B_ref(x, B_w_gate, B_w_up, B_w_down)
    return g * a + (1 - g) * b
```

```python
import jax
import jax.numpy as jnp
from jax.experimental import pallas as pl
import jax.experimental.pallas.tpu as pltpu

SEG = 32
HG = 4
GROUPS = (4, 4, 4, 4, 4, 4, 4, 4)
SPB = 8
FM = 256


def _gelu(x):
    c = 0.7978845608028654
    return 0.5 * x * (1.0 + jnp.tanh(c * (x + 0.044715 * (x * x * x))))


@jax.jit
def pallas_gated_mix__memory_aug_recurrent_mem_tr__glu_gated_geglu__prompt_kernel(
    A_x, A_mem0, A_Wq, A_Wk, A_Wv, A_Wo, A_seg_len, B_x, B_w_gate, B_w_up, B_w_down, gate_w,
):
    _, S, D = A_x.shape
    M = A_mem0.shape[1]
    H, E = A_Wq.shape[1], A_Wq.shape[2]
    F = B_w_gate.shape[1]
    L = M + SEG
    n_seg = S // SEG
    RB = SPB * SEG
    scale = float(E) ** -0.5
    NG = len(GROUPS)
    gb = [sum(GROUPS[:g]) for g in range(NG + 1)]
    GW = HG * E
    bf = jnp.bfloat16
    f32 = jnp.float32
    NT = (((1,), (1,)), ((), ()))

    def mm(a, b):
        return jax.lax.dot_general(a, b, (((1,), (0,)), ((), ())), preferred_element_type=f32)

    def rnd(a):
        return a.astype(bf).astype(f32)

    def kern(x_hbm, mem0_ref, wq_hbm, wk_hbm, wv_hbm, wo_hbm, wg_hbm, wu_hbm, wd_hbm, gw_ref,
             o_ref, x_v, wq3, wk3, wv3, wq, wk, wv, wo, wg, wu, wd, b_v, mem_v, sems):
        i = pl.program_id(0)

        @pl.when(i == 0)
        def _():
            NR = S // FM
            DC = D // NR // 16
            cx = pltpu.make_async_copy(x_hbm, x_v, sems.at[0])
            cg = pltpu.make_async_copy(wg_hbm, wg, sems.at[1])
            cu = pltpu.make_async_copy(wu_hbm, wu, sems.at[2])
            cd = pltpu.make_async_copy(wd_hbm, wd, sems.at[3])
            co = pltpu.make_async_copy(wo_hbm, wo, sems.at[4])
            bounds = [min(c * DC * 16, D) for c in range(NR + 1)]

            def wcopies(c):
                lo, n = bounds[c], bounds[c + 1] - bounds[c]
                return [pltpu.make_async_copy(s_.at[pl.ds(lo, n)], d_.at[pl.ds(lo, n)], sems.at[5 + 3 * c + t])
                        for t, (s_, d_) in enumerate(((wq_hbm, wq3), (wk_hbm, wk3), (wv_hbm, wv3)))]
            for c in (cg, cx, cu, cd):
                c.start()
            for c in range(NR):
                for cp in wcopies(c):
                    cp.start()
            co.start()
            mem_v[...] = mem0_ref[...]
            for c in (cg, cx, cu, cd):
                c.wait()

            def ffn(r, carry):
                for c in range(NR):
                    @pl.when(r == c)
                    def _():
                        for cp in wcopies(c):
                            cp.wait()
                r0 = pl.multiple_of(r * FM, FM)
                xb = x_v[pl.ds(r0, FM), :]
                g = jax.lax.dot_general(xb, wg[...], NT, preferred_element_type=f32)
                u = jax.lax.dot_general(xb, wu[...], NT, preferred_element_type=f32)
                hh = (_gelu(g) * u).astype(bf)
                b_v[pl.ds(r0, FM), :] = jnp.dot(hh, wd[...], preferred_element_type=f32)
                for t in range(DC):
                    ch = r * DC + t
                    d0 = pl.multiple_of(ch * 16, 16)
                    for w3, w2 in ((wq3, wq), (wk3, wk), (wv3, wv)):
                        w2[ch] = w3[pl.ds(d0, 16)].reshape(16, H * E)
                return carry
            jax.lax.fori_loop(0, NR, ffn, 0)
            co.wait()

        row = jax.lax.broadcasted_iota(jnp.int32, (L, L), 0)
        col = jax.lax.broadcasted_iota(jnp.int32, (L, L), 1)
        mask = (row < M) | (row >= col)

        def seg(j, mem):
            l0 = pl.multiple_of(j * SEG, SEG)
            r0 = pl.multiple_of(i * RB + j * SEG, SEG)
            xs = x_v[pl.ds(r0, SEG), :]
            h = jnp.concatenate([mem, xs.astype(f32)], axis=0)
            def proj(w, g):
                return mm(h, w[:, :, gb[g] * E:gb[g + 1] * E].reshape(D, GROUPS[g] * E))

            def attn(q, k, v, a):
                hs = slice(a * E, (a + 1) * E)
                s = jax.lax.dot_general(rnd(q[:, hs]), k[:, hs].astype(bf), NT,
                                        preferred_element_type=f32) * scale
                s = jnp.where(mask, s, -1e9)
                e = jnp.exp(s - jnp.max(s, axis=-1, keepdims=True))
                p = e / jnp.sum(e, axis=-1, keepdims=True)
                return rnd(mm(rnd(p), v[:, hs].astype(bf)))

            acc = None
            qkv = None
            og = None
            for g in range(NG + 2):
                new = [None] * 3
                os_ = []
                parts = [("p", 0), ("p", 1), ("p", 2), ("o", 0)]
                for n, (kind, idx) in enumerate(parts):
                    if kind == "p":
                        if g < NG:
                            new[idx] = proj((wq, wk, wv)[idx], g)
                    elif og is not None:
                        y = mm(og, wo[gb[g - 2] * E:gb[g - 1] * E, :])
                        acc = y if acc is None else acc + y
                    if qkv is not None:
                        for a in range(-(-n * GROUPS[g - 1] // 4), -(-(n + 1) * GROUPS[g - 1] // 4)):
                            os_.append(attn(*qkv, a))
                og = jnp.concatenate(os_, axis=1) if os_ else None
                qkv = new if g < NG else None
            xf = xs.astype(f32)
            gate = jax.nn.sigmoid(jnp.sum(xf * gw_ref[...].astype(f32).reshape(1, D), axis=-1, keepdims=True))
            o_ref[pl.ds(l0, SEG), :] = (gate * acc[M:] + (1.0 - gate) * b_v[pl.ds(r0, SEG), :]).astype(o_ref.dtype)
            return rnd(acc[:M])
        mem_v[...] = jax.lax.fori_loop(0, SPB, seg, mem_v[...].astype(f32)).astype(bf)

    anyspec = pl.BlockSpec(memory_space=pl.ANY)
    out = pl.pallas_call(
        kern,
        grid=(n_seg // SPB,),
        in_specs=[anyspec, pl.BlockSpec((M, D), lambda i: (0, 0))] + [anyspec] * 7
        + [pl.BlockSpec((D,), lambda i: (0,))],
        out_specs=pl.BlockSpec((RB, D), lambda i: (i, 0)),
        out_shape=jax.ShapeDtypeStruct((S, D), A_x.dtype),
        scratch_shapes=[
            pltpu.VMEM((S, D), bf),
            pltpu.VMEM((D, H, E), bf), pltpu.VMEM((D, H, E), bf), pltpu.VMEM((D, H, E), bf),
            pltpu.VMEM((D // 16, 16, H * E), bf), pltpu.VMEM((D // 16, 16, H * E), bf),
            pltpu.VMEM((D // 16, 16, H * E), bf),
            pltpu.VMEM((H * E, D), bf),
            pltpu.VMEM((F, D), bf), pltpu.VMEM((F, D), bf), pltpu.VMEM((F, D), bf),
            pltpu.VMEM((S, D), f32),
            pltpu.VMEM((M, D), bf),
            pltpu.SemaphoreType.DMA((5 + 3 * (S // FM),)),
        ],
        compiler_params=pltpu.CompilerParams(
            dimension_semantics=("arbitrary",), vmem_limit_bytes=100 * 2**20),
    )(A_x.reshape(S, D), A_mem0.reshape(M, D), A_Wq, A_Wk,
      A_Wv, A_Wo.reshape(H * E, D), B_w_gate.T, B_w_up.T, B_w_down, gate_w)
    return out.reshape(1, S, D)
```
